```python
import os as _os
_os.environ.setdefault('JAX_PLATFORMS', 'cpu')
import jax
import jax.numpy as jnp

def _softmax(x, axis=-1):
    return jax.nn.softmax(x, axis=axis)

def _gelu(x):
    return jax.nn.gelu(x, approximate=True)

def _silu(x):
    return jax.nn.silu(x)

def _sigmoid(x):
    return jax.nn.sigmoid(x)

def _layernorm(x, axis=-1, eps=1e-05):
    m = jnp.mean(x, axis=axis, keepdims=True)
    v = jnp.var(x, axis=axis, keepdims=True)
    return (x - m) / jnp.sqrt(v + eps)

def _scatter_add(tgt, idx, src, axis=0):
    return tgt.at[idx].add(src)

def _segment_sum(src, seg, n):
    return jax.ops.segment_sum(src, seg, n)

class _Rng:

    def __init__(self, key):
        self._k = key

    def _next(self):
        self._k, sub = jax.random.split(self._k)
        return sub

    def normal(self, shape):
        return jax.random.normal(self._next(), shape, dtype=jnp.bfloat16)

    def randint(self, lo, hi, shape):
        return jax.random.randint(self._next(), shape, lo, hi, dtype=jnp.int32)

    def uniform(self, shape, lo=0.0, hi=1.0):
        return jax.random.uniform(self._next(), shape, jnp.bfloat16, lo, hi)

    def permutation(self, n):
        return jax.random.permutation(self._next(), n)
kernel_name = 'standalone__window_attn_twins__vision'

def setup_inputs():
    _rng = _Rng(jax.random.key(int.from_bytes(__import__("os").urandom(4), "little")))
    _w = lambda a: (lambda t: t.astype(jnp.bfloat16) if jnp.issubdtype(t.dtype, jnp.floating) else t)(jnp.asarray(a))
    H = W = 384 // 8 * 8
    C = 96
    return {'x': _w((lambda *s: _rng.normal(s) * 0.4)(1, H, W, C)), 'wq': _w((lambda *s: _rng.normal(s) * 0.4)(C, C)), 'wkv': _w((lambda *s: _rng.normal(s) * 0.4)(C, 2 * C)), 'wo': _w((lambda *s: _rng.normal(s) * 0.05)(C, C))}

def reference(x, wq, wkv, wo):
    B, H, W, C = x.shape
    win = 8
    nh, nw = (H // win, W // win)
    xs = x.reshape(B, nh, win, nw, win, C).mean(axis=(2, 4)).reshape(B, nh * nw, C)
    q = x.reshape(B, H * W, C) @ wq
    kv = xs @ wkv
    k, v = (kv[..., :C].copy(), kv[..., C:].copy())
    scale = C ** (-0.5)
    p = _softmax(jnp.einsum('bqc,bkc->bqk', q, k) * scale, axis=-1)
    o = jnp.einsum('bqk,bkc->bqc', p, v) @ wo
    return o.reshape(B, H, W, C)
```

```python
import functools

import jax
import jax.numpy as jnp
import jax.experimental.pallas as pl
import jax.experimental.pallas.tpu as pltpu

WIN = 8
LOG2E = 1.4426950408889634
KC = 128
RPI = 12
SK = 2
LAG = 3
ODMA = 2
NV = 2
TV = 6
CPS = 12
VLAG = 3
RF = 35
LAGU = 2
LAG0 = 3
SLAB = 24
WS = 14
CH_WINS = (3, 3, 2)
CH_OFF = (0, 3, 6)

_NT = (((1,), (1,)), ((), ()))


def _kernel(x_hbm, wq_hbm, wkv_hbm, wo_hbm, o_hbm,
            x_ref, o_ref, kq_ref, vot_ref, w_ref, s0_ref, s1_ref,
            acc_ref, m_ref, l_ref, kb_ref, wq_ref, wkv_ref, wo_ref, in_sems, w_sems, out_sem, *, C, H, W):
    f32, bf16 = jnp.float32, jnp.bfloat16
    NT = (H // WIN) * (W // WIN) // KC
    ND = NT // 3
    LT = W // 128

    def in_copy(d, j):
        row0 = (d * 8 + CH_OFF[j]) * WIN
        n = CH_WINS[j] * WIN
        return pltpu.make_async_copy(x_hbm.at[pl.ds(row0, n)], x_ref.at[pl.ds(row0, n)],
                                     in_sems.at[d * 3 + j])

    def out_copy(row0, n):
        return pltpu.make_async_copy(o_ref.at[pl.ds(row0, n)], o_hbm.at[pl.ds(row0, n)], out_sem)

    w_copies = [pltpu.make_async_copy(s, t, w_sems.at[i]) for i, (s, t) in
                enumerate(((wq_hbm, wq_ref), (wkv_hbm, wkv_ref), (wo_hbm, wo_ref)))]
    for cp in w_copies:
        cp.start()
    for d in range(ND):
        for j in range(3):
            in_copy(d, j).start(priority=1)

    def init(r, carry):
        acc_ref[r] = jnp.zeros((C, W), f32)
        l_ref[r] = jnp.zeros((8, W), f32)
        m_ref[r] = jnp.full((8, W), -jnp.inf, f32)
        return carry

    jax.lax.fori_loop(0, RF, init, 0)
    m_ref[RF] = jnp.full((8, W), -jnp.inf, f32)
    for cp in w_copies:
        cp.wait()
    w_ref[0] = (jax.lax.dot_general(wq_ref[...], wkv_ref[:, :C], _NT, preferred_element_type=f32)
                * (C ** -0.5 * LOG2E)).astype(bf16)
    w_ref[1] = jnp.dot(wkv_ref[:, C:], wo_ref[...], preferred_element_type=f32).T.astype(bf16)

    def prep(d, j):
        blocks = [(b // LT, b % LT) for b in range(8 * j, 8 * j + 8)]

        def colsum(blk, sl):
            w, lt = blk
            xr = x_ref[pl.ds((d * 8 + w) * WIN, WIN), sl, lt * 128:(lt + 1) * 128]
            return jnp.sum(xr.astype(f32), axis=0)

        def merge(a, b, k):
            lane = jax.lax.broadcasted_iota(jnp.int32, a.shape, 1)
            return jnp.where((lane & k) == 0, a + pltpu.roll(a, 128 - k, 1), b + pltpu.roll(b, k, 1))

        xst = []
        for sb in range(C // SLAB):
            sl = slice(sb * SLAB, (sb + 1) * SLAB)
            lv = []
            for p in range(4):
                lv.append(merge(colsum(blocks[2 * p], sl), colsum(blocks[2 * p + 1], sl), 1))
                if p == 1:
                    lv = [merge(lv[0], lv[1], 2)]
                if p == 3:
                    lv = [merge(lv[0], merge(lv[1], lv[2], 2), 4)]
                yield jnp.concatenate([lv[-1][8 * q:8 * q + 8] for q in range(LT)], axis=1)
            xst.append(lv[0])
        xst = (jnp.concatenate(xst, axis=0) * (1.0 / (WIN * WIN))).astype(bf16)
        t = d * 3 + j
        kq_ref[t] = jnp.dot(w_ref[0], xst, preferred_element_type=f32).T.astype(bf16)
        vot_ref[t] = jnp.dot(w_ref[1], xst, preferred_element_type=f32).astype(bf16)
        yield None

    def part_max(sc):
        return jnp.max(sc.reshape(KC // 8, 8, W), axis=0)

    def part_sum(p):
        n = p.shape[0] // 2
        p = jnp.sum(p.reshape(n, 2, 8, W), axis=1).reshape(n * 8, W)
        acc = p[8 * (n - 1):]
        for i in range(n - 2, -1, -1):
            acc = acc + p[8 * i:8 * i + 8]
        return acc

    def fin_max(m8):
        return jnp.broadcast_to(jnp.max(m8, axis=0, keepdims=True), (8, W))

    def tie(m, g):
        return jnp.maximum(m, jnp.minimum(m, g))

    def normalize(acc, l8):
        return (acc / jnp.sum(l8, axis=0, keepdims=True)).astype(o_ref.dtype)

    in_copy(0, 0).wait()
    for _ in prep(0, 0):
        pass

    NSTEP = 4 * (C // SLAB) + 1
    assert SLAB == 8 * LT and WS < CH_WINS[0] * WIN and RF + 1 < (CH_WINS[0] + CH_WINS[1]) * WIN
    assert WS + NSTEP < RF

    def online_body(d, carry):
        scores, gates = [], []

        def finish():
            r, s, vot_t = scores.pop(0)
            m_old = m_ref[r]
            m_new = jnp.maximum(m_old, fin_max(part_max(s)))
            mg = m_new
            while gates:
                mg = tie(mg, gates.pop(0))
            alpha = jnp.exp2(m_old - m_new)
            p = jnp.exp2(s.reshape(KC // 8, 8, W) - mg[None])
            l_ref[r] = l_ref[r] * alpha + part_sum(p)
            m_ref[r] = m_new
            pv = jnp.dot(vot_t, p.reshape(KC, W).astype(bf16), preferred_element_type=f32)
            acc_ref[r] = (acc_ref[r].reshape(C // 8, 8, W) * alpha[None]).reshape(C, W) + pv

        for j in range(3):
            t = d * 3 + j
            kq_t = kq_ref[t]
            vot_t = vot_ref[t]
            nxt = prep(d, j + 1) if j < 2 else prep(jnp.minimum(d + 1, ND - 1), 0)
            p0 = WS + 1 if j < 2 else LAG0
            for i in range(RF + 1):
                sc = jnp.dot(kq_t, x_ref[i], preferred_element_type=f32)
                if i < RF:
                    scores.append((i, sc, vot_t))
                else:
                    s0_ref[pl.ds(pl.multiple_of(t * KC, KC), KC), :] = sc
                    m_ref[RF] = jnp.maximum(m_ref[RF], part_max(sc))
                if p0 <= i < p0 + NSTEP:
                    g = next(nxt)
                    if g is not None:
                        gates.append(g)
                if i == WS and j < 2:
                    in_copy(d, j + 1).wait()
                    if j == 1:
                        @pl.when(d + 1 < ND)
                        def _():
                            in_copy(d + 1, 0).wait()
                lag = LAG0 if (j == 0 and i <= LAG0) else LAGU
                for _ in range(2):
                    if len(scores) > lag:
                        finish()
        while scores:
            finish()
        return carry

    jax.lax.fori_loop(0, ND, online_body, 0)

    def pv_chunk(s_r, mb, c, acc, l8):
        p = jnp.exp2(s_r[c * KC:(c + 1) * KC, :].reshape(KC // 8, 8, W) - mb[None])
        lc = part_sum(p)
        oc = jnp.dot(vot_ref[c], p.reshape(KC, W).astype(bf16), preferred_element_type=f32)
        if acc is None:
            return oc, lc
        return acc + oc, l8 + lc

    def qk_chunk(xt, s_w, c, m8):
        n = KC - 8 * NV if c == TV else KC
        sc = jnp.dot(kq_ref[c, :n, :], xt, preferred_element_type=f32)
        s_w[c * KC:c * KC + n, :] = sc
        mc = jnp.max(sc.reshape(n // 8, 8, W), axis=0)
        return mc if m8 is None else jnp.maximum(m8, mc)

    def vpu_scores(row, s_w):
        for g in range(NV):
            acc = None
            for c0 in range(0, C, CPS):
                xn = {j: x_ref[row, 8 * j:8 * j + 8, :].astype(f32)
                      for j in range(c0 // 8, (c0 + CPS - 1) // 8 + 1)}
                xb = jnp.concatenate([jnp.broadcast_to(xn[c // 8][c % 8:c % 8 + 1, :], (8, W))
                                      for c in range(c0, c0 + CPS)], axis=0).reshape(CPS, 8, W)
                kb = kb_ref[g * C + c0:g * C + c0 + CPS]
                terms = jnp.concatenate([kb] * LT, axis=2) * xb
                if acc is not None:
                    terms = jnp.concatenate([acc[None], terms], axis=0)
                acc = jnp.sum(terms, axis=0)
                if c0 + CPS == C:
                    r = (TV + 1) * KC - 8 * (NV - g)
                    s_w[r:r + 8, :] = acc
                yield acc, c0 + CPS == C

    bufs = (s0_ref, s1_ref)
    NIT = (H - RF - 1) // RPI
    NPER = -(-RF // (NIT - 2))
    NVS = NV * C // CPS
    assert RPI % 2 == 0 and RPI % ODMA == 0 and RF + 1 + NIT * RPI == H and NPER * LT <= RPI
    assert C % CPS == 0 and NVS <= NT - SK and TV >= SK and NV % 2 == 0

    m8 = None
    for c in range(SK):
        m8 = qk_chunk(x_ref[RF + 1], s1_ref, c, m8)
    mb = fin_max(m_ref[RF])
    ksel = kq_ref[TV, KC - 8 * NV:, :].astype(f32)
    for c in range(C):
        kc = jnp.broadcast_to(ksel[:, c:c + 1], (8 * NV, 128))
        for g in range(NV):
            kb_ref[g * C + c] = kc[8 * g:8 * g + 8]

    def body(it, carry):
        mb, m8 = carry
        r0 = RF + it * RPI
        hist, vhist = [], []
        x1 = x_ref[r0 + 1]
        for u in range(RPI):
            if u + 1 < RPI:
                x2 = x_ref[r0 + u + 2]
            else:
                x2 = x_ref[jnp.minimum(r0 + u + 2, H - 1)]
            acc = l8 = m_next = None
            vgen = vpu_scores(r0 + u + 1, bufs[(u + 1) % 2])
            for c in range(NT):
                cq = c + SK
                sv = None
                if c < NVS:
                    sv, complete = next(vgen)
                    if complete:
                        m8 = jnp.maximum(m8, sv)
                vhist.append(sv)
                if cq < NT:
                    m8 = qk_chunk(x1, bufs[(u + 1) % 2], cq, m8)
                    if cq == NT - 1:
                        m_next = fin_max(m8)
                else:
                    m8 = qk_chunk(x2, bufs[u % 2], cq - NT, None if cq == NT else m8)
                hist.append(m8)
                mg = tie(mb, hist[-1 - LAG]) if len(hist) > LAG else mb
                if len(vhist) > VLAG and vhist[-1 - VLAG] is not None:
                    mg = tie(mg, vhist[-1 - VLAG])
                acc, l8 = pv_chunk(bufs[u % 2], mg, c, acc, l8)
            if u < NPER * LT:
                r = it * NPER + u // LT
                rr = jnp.minimum(r, RF - 1)
                ls = slice((u % LT) * 128, (u % LT + 1) * 128)
                o_ref[jnp.where(r < RF, r, H), :, ls] = normalize(acc_ref[rr, :, ls], l_ref[rr, :, ls])
                if u == NPER * LT - 1:
                    @pl.when(it == (RF - 1) // NPER)
                    def _():
                        out_copy(0, RF).start()
            o_ref[r0 + u] = normalize(acc, l8)
            mb = m_next
            x1 = x2
            if (u + 1) % ODMA == 0:
                out_copy(r0 + u + 1 - ODMA, ODMA).start()
        return mb, m8

    mb, _ = jax.lax.fori_loop(0, NIT, body, (mb, m8))
    acc = l8 = None
    for c in range(NT):
        acc, l8 = pv_chunk(s0_ref, mb, c, acc, l8)
    o_ref[H - 1] = normalize(acc, l8)
    out_copy(H - 1, 1).start()
    out_copy(0, H).wait()


@jax.jit
def pallas_standalone__window_attn_twins__vision_kernel(
    x: jax.Array,
    wq: jax.Array,
    wkv: jax.Array,
    wo: jax.Array,
):
    B, H, W, C = x.shape
    assert B == 1
    NK = (H // WIN) * (W // WIN)
    xt = jnp.transpose(x, (0, 1, 3, 2)).reshape(H, C, W)
    out = pl.pallas_call(
        functools.partial(_kernel, C=C, H=H, W=W),
        in_specs=[pl.BlockSpec(memory_space=pl.ANY)] * 4,
        out_specs=pl.BlockSpec(memory_space=pl.ANY),
        out_shape=jax.ShapeDtypeStruct((H, C, W), x.dtype),
        scratch_shapes=[
            pltpu.VMEM((H, C, W), x.dtype),
            pltpu.VMEM((H + 1, C, W), x.dtype),
            pltpu.VMEM((NK // KC, KC, C), jnp.bfloat16),
            pltpu.VMEM((NK // KC, C, KC), jnp.bfloat16),
            pltpu.VMEM((2, C, C), jnp.bfloat16),
            pltpu.VMEM((NK, W), jnp.float32),
            pltpu.VMEM((NK, W), jnp.float32),
            pltpu.VMEM((RF, C, W), jnp.float32),
            pltpu.VMEM((RF + 1, 8, W), jnp.float32),
            pltpu.VMEM((RF, 8, W), jnp.float32),
            pltpu.VMEM((NV * C, 8, 128), jnp.float32),
            pltpu.VMEM((C, C), wq.dtype),
            pltpu.VMEM((C, 2 * C), wkv.dtype),
            pltpu.VMEM((C, C), wo.dtype),
            pltpu.SemaphoreType.DMA((NK // KC,)),
            pltpu.SemaphoreType.DMA((3,)),
            pltpu.SemaphoreType.DMA(()),
        ],
        compiler_params=pltpu.CompilerParams(
            vmem_limit_bytes=110 * 1024 * 1024,
            disable_bounds_checks=True,
        ),
    )(xt, wq, wkv, wo)
    return jnp.transpose(out.reshape(B, H, C, W), (0, 1, 3, 2))
```
